```python
import jax
import jax.numpy as jnp

def _softmax(x, axis=-1):
    return jax.nn.softmax(x, axis=axis)

def _gelu(x):
    return jax.nn.gelu(x, approximate=True)

def _silu(x):
    return jax.nn.silu(x)

def _sigmoid(x):
    return jax.nn.sigmoid(x)

def _layernorm(x, axis=-1, eps=1e-05):
    m = jnp.mean(x, axis=axis, keepdims=True)
    v = jnp.var(x, axis=axis, keepdims=True)
    return (x - m) / jnp.sqrt(v + eps)

def _scatter_add(tgt, idx, src, axis=0):
    return tgt.at[idx].add(src)

def _segment_sum(src, seg, n):
    return jax.ops.segment_sum(src, seg, n)

class _Rng:

    def __init__(self, key):
        self._k = key

    def _next(self):
        self._k, sub = jax.random.split(self._k)
        return sub

    def normal(self, shape):
        return jax.random.normal(self._next(), shape, dtype=jnp.bfloat16)

    def randint(self, lo, hi, shape):
        return jax.random.randint(self._next(), shape, lo, hi, dtype=jnp.int32)

    def uniform(self, shape, lo=0.0, hi=1.0):
        return jax.random.uniform(self._next(), shape, jnp.bfloat16, lo, hi)

    def permutation(self, n):
        return jax.random.permutation(self._next(), n)
kernel_name = 'adaLN_cond__gqa_block_cached__moe_arch_mod__decode'

def setup_inputs():
    _rng = _Rng(jax.random.key(int.from_bytes(__import__("os").urandom(4), "little")))
    _w = lambda a: (lambda t: t.astype(jnp.bfloat16) if jnp.issubdtype(t.dtype, jnp.floating) else t)(jnp.asarray(a))

    def _A_setup():
        B, Sq, D = (4, 1, 512)
        Hq, Hkv, Sk, Dh = (32, 32, 8192, 128)
        assert Hq % Hkv == 0, (Hq, Hkv)
        return {'x': _w((lambda *s: _rng.normal(s) * 0.05)(B, Sq, D)), 'k_cache': _w((lambda *s: _rng.normal(s) * 0.05)(B, Hkv, Sk, Dh)), 'v_cache': _w((lambda *s: _rng.normal(s) * 0.05)(B, Hkv, Sk, Dh)), 'wq': _w((lambda *s: _rng.normal(s) * 0.05)(D, Hq * Dh) * D ** (-0.5)), 'wo': _w((lambda *s: _rng.normal(s) * 0.05)(Hq * Dh, D) * (Hq * Dh) ** (-0.5))}
    _A_in = _A_setup()

    def _B_setup():
        B, S, D, F, C = (4, 1, 512, 1376, 1)
        return {'x': _w((lambda *s: _rng.normal(s) * 0.05)(B, S, D)), 'w_r': _w((lambda *s: _rng.normal(s) * 0.05)(D)), 'w_gate': _w((lambda *s: _rng.normal(s) * 0.05)(D, F)), 'w_up': _w((lambda *s: _rng.normal(s) * 0.05)(D, F)), 'w_down': _w((lambda *s: _rng.normal(s) * 0.05)(F, D))}
    _B_in = _B_setup()
    return {'A_x': _A_in['x'], 'A_k_cache': _A_in['k_cache'], 'A_v_cache': _A_in['v_cache'], 'A_wq': _A_in['wq'], 'A_wo': _A_in['wo'], 'B_x': _B_in['x'], 'B_w_r': _B_in['w_r'], 'B_w_gate': _B_in['w_gate'], 'B_w_up': _B_in['w_up'], 'B_w_down': _B_in['w_down'], 'c': _w((lambda *s: _rng.normal(s) * 0.05)(4, 512)), 'w_mod': _w((lambda *s: _rng.normal(s) * 0.05)(512, 6 * 512) * 512 ** (-0.5))}

def reference(A_x, A_k_cache, A_v_cache, A_wq, A_wo, B_x, B_w_r, B_w_gate, B_w_up, B_w_down, c, w_mod):

    def _A_ref(x, k_cache, v_cache, wq, wo):
        B, Sq, D = x.shape
        Hq, Dh = (32, 128)
        Hkv = k_cache.shape[1]
        rep = Hq // Hkv
        q = (lambda x, *d: x.transpose(*d))((x @ wq).reshape(B, Sq, Hq, Dh), 0, 2, 1, 3)
        k = jnp.repeat(k_cache, rep, axis=1)
        v = jnp.repeat(v_cache, rep, axis=1)
        scores = jnp.einsum('bhqd,bhkd->bhqk', q, k) * Dh ** (-0.5)
        p = _softmax(scores, axis=-1)
        o = jnp.einsum('bhqk,bhkd->bhqd', p, v)
        return (lambda x, *d: x.transpose(*d))(o, 0, 2, 1, 3).reshape(B, Sq, Hq * Dh) @ wo

    def _B_ref(x, w_r, w_gate, w_up, w_down):
        B, S, D = x.shape
        C = 1
        r = x @ w_r
        idx = jnp.argsort(-r, axis=-1)[:, :C]
        idx_e = jnp.repeat(idx.reshape(B, C, 1), D, axis=2)
        x_sel = jnp.take_along_axis(x, idx_e, axis=1)
        g = _silu(x_sel @ w_gate)
        u = x_sel @ w_up
        y = g * u @ w_down
        r_sel = _sigmoid(jnp.take_along_axis(r, idx, axis=1))
        y = y * r_sel.reshape(B, C, 1)
        b_off = (jnp.arange(B) * S).reshape(B, 1)
        flat_idx = (idx + b_off).reshape(B * C)
        zero = (x * 0.0).reshape(B * S, D)
        upd = _scatter_add(zero, flat_idx, y.reshape(B * C, D), axis=0)
        return x + upd.reshape(B, S, D)
    x = A_x
    mod = (_silu(c) @ w_mod).reshape(c.shape[0], 6, 1, -1)
    sa, ca, ga, sb, cb, gb = (mod[:, 0].copy(), mod[:, 1].copy(), mod[:, 2].copy(), mod[:, 3].copy(), mod[:, 4].copy(), mod[:, 5].copy())
    h = _layernorm(x, axis=-1) * (1 + ca) + sa
    x = x + ga * _A_ref(h, A_k_cache, A_v_cache, A_wq, A_wo)
    h = _layernorm(x, axis=-1) * (1 + cb) + sb
    x = x + gb * _B_ref(h, B_w_r, B_w_gate, B_w_up, B_w_down)
    return x
```

```python
import functools

import jax
import jax.numpy as jnp
import jax.experimental.pallas as pl
import jax.experimental.pallas.tpu as pltpu

F32 = jnp.float32
BF16 = jnp.bfloat16


def make_pattern(S, ch, nstream):
    reg = S // nstream
    out = []
    for i in range(-(-reg // ch)):
        for s in range(nstream):
            out.append((s * reg + i * ch, min(ch, reg - i * ch)))
    return out


def build(nbuf=3, ch=128, nstream=4, order="hb", issue="end", small="manual"):
    def fn(A_x, A_k_cache, A_v_cache, A_wq, A_wo, B_x, B_w_r, B_w_gate, B_w_up, B_w_down, c, w_mod):
        del B_x
        B, H, S, Dh = A_k_cache.shape
        D = A_x.shape[-1]
        F = B_w_gate.shape[-1]
        NH = B * H
        pat = make_pattern(S, ch, nstream)
        scale = Dh ** -0.5

        def layernorm(x):
            m = jnp.mean(x, axis=-1, keepdims=True)
            xc = x - m
            v = jnp.mean(xc * xc, axis=-1, keepdims=True)
            return xc / jnp.sqrt(v + 1e-5)

        def silu(x):
            return x / (1.0 + jnp.exp(-x))

        def kernel(x_hbm, c_hbm, wmod_hbm, wq_hbm, wo_hbm, wr_hbm, wg_hbm, wu_hbm, wd_hbm, k_hbm, v_hbm,
                   o_ref,
                   x_v, c_v, wmod_v, wq_v, wo_v, wr_v, wg_v, wu_v, wd_v, kbuf, vbuf, q_scr, mod_scr,
                   wsem, kvsem):
            def bh(i):
                if order == "hb":
                    return i % B, i // B
                return i // H, i % H

            def start_kv(i, slot):
                b, h = bh(i)
                for (r0, nr) in pat:
                    pltpu.make_async_copy(k_hbm.at[b, h, pl.ds(r0, nr)], kbuf.at[slot, pl.ds(r0, nr)],
                                          kvsem.at[0, slot]).start(priority=0)
                    pltpu.make_async_copy(v_hbm.at[b, h, pl.ds(r0, nr)], vbuf.at[slot, pl.ds(r0, nr)],
                                          kvsem.at[1, slot]).start(priority=1)

            def wait_k(slot):
                pltpu.make_async_copy(kbuf.at[slot], kbuf.at[slot], kvsem.at[0, slot]).wait()

            def wait_v(slot):
                pltpu.make_async_copy(vbuf.at[slot], vbuf.at[slot], kvsem.at[1, slot]).wait()

            smalls = [(c_hbm, c_v), (wmod_hbm, wmod_v), (x_hbm, x_v), (wq_hbm, wq_v), (wo_hbm, wo_v),
                      (wr_hbm, wr_v), (wg_hbm, wg_v), (wu_hbm, wu_v), (wd_hbm, wd_v)]
            cps = [pltpu.make_async_copy(s, d, wsem.at[j]) for j, (s, d) in enumerate(smalls)]
            for j in range(4):
                cps[j].start()
            start_kv(0, 0)
            cps[4].start()
            for s in range(1, nbuf):
                start_kv(s, s)
            for j in range(5, 9):
                cps[j].start()

            cps[0].wait()
            cps[1].wait()
            cs = silu(c_v[...].astype(F32)).astype(BF16)
            mod = jnp.dot(cs, wmod_v[...], preferred_element_type=F32)
            mod = mod.astype(BF16).astype(F32)
            mod_scr[...] = mod
            cps[2].wait()
            x = x_v[...].astype(F32)
            sa, ca = mod[:, 0:D], mod[:, D:2 * D]
            h1 = (layernorm(x) * (1.0 + ca) + sa).astype(BF16)
            cps[3].wait()
            q = jnp.dot(h1, wq_v[...], preferred_element_type=F32).astype(BF16)
            for hd in range(H):
                q_scr[hd] = q[:, hd * Dh:(hd + 1) * Dh]
            cps[4].wait()

            row = jax.lax.broadcasted_iota(jnp.int32, (B, Dh), 0)

            def body(i, acc):
                slot = i % nbuf
                b, h = bh(i)
                wait_k(slot)
                wait_v(slot)
                qh = q_scr[h]
                s = jax.lax.dot_general(qh, kbuf[slot], (((1,), (1,)), ((), ())), preferred_element_type=F32)
                m = jnp.max(s, axis=1, keepdims=True)
                p = jnp.exp((s - m) * scale)
                l = jnp.sum(p, axis=1, keepdims=True)
                o = jnp.dot(p.astype(BF16), vbuf[slot], preferred_element_type=F32)

                @pl.when(i + nbuf < NH)
                def _():
                    start_kv(i + nbuf, slot)

                o = jnp.where(row == b, o / l, 0.0).astype(BF16)
                wo_h = wo_v[pl.ds(pl.multiple_of(h * Dh, Dh), Dh), :]
                return acc + jnp.dot(o, wo_h, preferred_element_type=F32)

            attn = jax.lax.fori_loop(0, NH, body, jnp.zeros((B, D), F32))

            for j in range(5, 9):
                cps[j].wait()
            mod = mod_scr[...]
            ga, sb, cb, gb = (mod[:, j * D:(j + 1) * D] for j in range(2, 6))
            x = x_v[...].astype(F32)
            x1 = x + ga * attn
            h2 = layernorm(x1) * (1.0 + cb) + sb
            h2b = h2.astype(BF16)
            r = jnp.sum(h2b.astype(F32) * wr_v[...].astype(F32).reshape(1, D), axis=-1, keepdims=True)
            g = jax.lax.dot_general(h2b, wg_v[...], (((1,), (1,)), ((), ())), preferred_element_type=F32)
            u = jax.lax.dot_general(h2b, wu_v[...], (((1,), (1,)), ((), ())), preferred_element_type=F32)
            a = (silu(g) * u).astype(BF16)
            y = jnp.dot(a, wd_v[...], preferred_element_type=F32)
            y = y * (1.0 / (1.0 + jnp.exp(-r)))
            upd = h2 * 0.0 + y
            out = x1 + gb * (h2 + upd)
            o_ref[...] = out.astype(o_ref.dtype)

        any_spec = pl.BlockSpec(memory_space=pltpu.HBM if small == 'manual' else pl.ANY)
        out = pl.pallas_call(
            kernel,
            out_shape=jax.ShapeDtypeStruct((B, D), A_x.dtype),
            in_specs=[any_spec] * 11,
            out_specs=pl.BlockSpec(memory_space=pltpu.VMEM),
            scratch_shapes=[
                pltpu.VMEM((B, D), BF16), pltpu.VMEM(c.shape, BF16), pltpu.VMEM(w_mod.shape, BF16),
                pltpu.VMEM(A_wq.shape, BF16), pltpu.VMEM(A_wo.shape, BF16), pltpu.VMEM(B_w_r.shape, BF16),
                pltpu.VMEM((F, D), BF16), pltpu.VMEM((F, D), BF16), pltpu.VMEM(B_w_down.shape, BF16),
                pltpu.VMEM((nbuf, S, Dh), BF16), pltpu.VMEM((nbuf, S, Dh), BF16),
                pltpu.VMEM((H, B, Dh), BF16), pltpu.VMEM((B, 6 * D), F32),
                pltpu.SemaphoreType.DMA((9,)), pltpu.SemaphoreType.DMA((2, nbuf)),
            ],
            compiler_params=pltpu.CompilerParams(vmem_limit_bytes=100 * 1024 * 1024),
            name="fused_decode",
        )(A_x.reshape(B, D), c, w_mod, A_wq, A_wo, B_w_r, B_w_gate.T, B_w_up.T, B_w_down, A_k_cache, A_v_cache)
        return out.reshape(A_x.shape)

    return jax.jit(fn)


pallas_adaLN_cond__gqa_block_cached__moe_arch_mod__decode_kernel = build()
```

```python
import jax
import jax.numpy as jnp
import jax.experimental.pallas as pl
import jax.experimental.pallas.tpu as pltpu

F32 = jnp.float32
BF16 = jnp.bfloat16

Q = 4
LOOK = 2
CH = 80
W_ROWS = 32
W_COLS = 2048
W_STREAMS = 4
D_CUTS = (1152,)
EPS = 1e-5


def _layernorm(x):
    m = jnp.mean(x, axis=-1, keepdims=True)
    xc = x - m
    v = jnp.mean(xc * xc, axis=-1, keepdims=True)
    return xc / jnp.sqrt(v + EPS)


def _sigmoid(x):
    return 1.0 / (1.0 + jnp.exp(-x))


def _dot(a, b):
    return jnp.dot(a, b, preferred_element_type=F32)


def _dot_nt(a, b):
    return jax.lax.dot_general(a, b, (((1,), (1,)), ((), ())), preferred_element_type=F32)


def _pieces(src, dst, sem, rows, cols):
    n_rows, n_cols = src.shape
    out = []
    for r0 in range(0, n_rows, rows):
        nr = min(rows, n_rows - r0)
        for c0 in range(0, n_cols, cols):
            nc = min(cols, n_cols - c0)
            if nc == n_cols:
                out.append((src.at[pl.ds(r0, nr)], dst.at[pl.ds(r0, nr)], sem))
            else:
                out.append((src.at[pl.ds(r0, nr), pl.ds(c0, nc)],
                            dst.at[pl.ds(r0, nr), pl.ds(c0, nc)], sem))
    return out


def _streams(jobs, n):
    per = -(-len(jobs) // n)
    return [jobs[s * per + t] for t in range(per) for s in range(n) if s * per + t < len(jobs)]


def _interleave(*lists):
    out = []
    for t in range(max(len(l) for l in lists)):
        for l in lists:
            if t < len(l):
                out.append(l[t])
    return out


def _two_queues(jobs0, jobs1):
    return _interleave([[j + (0,)] for j in jobs0], [[j + (1,)] for j in jobs1])


def _halves(jobs):
    n = (len(jobs) + 1) // 2
    return _two_queues(_streams(jobs[:n], W_STREAMS), _streams(jobs[n:], W_STREAMS))


def _issue(groups):
    for group in groups:
        for src, dst, sem, queue in group:
            pltpu.make_async_copy(src, dst, sem).start(priority=queue)


def _wait_all(buf, sem):
    pltpu.make_async_copy(buf, buf, sem).wait()


def _make_kernel(B, H, S, Dh, D, F):
    n_heads = B * H
    part = S // Q
    n_slots = LOOK + Q - 1
    n_main = n_heads - n_slots
    first = -n_slots
    scale = Dh ** -0.5
    cuts = [0, *[c for c in D_CUTS if 0 < c < F], F]
    d_split = list(zip(cuts[:-1], cuts[1:]))

    def kernel(x_hbm, c_hbm, wmod_hbm, wq_hbm, wo_hbm, wr_hbm, wg_hbm, wu_hbm, wd_hbm, k_hbm, v_hbm,
               o_ref,
               x_v, c_v, wr_v, wmod_v, wq_v, wo_v, wg_v, wu_v, wd_v, kbuf, vbuf,
               q_scr, mod_scr, acc_scr, a_scr, wsem, kvsem, dsem):
        sem_c, sem_x, sem_r, sem_mod, sem_q, sem_o, sem_g, sem_u = (wsem.at[j] for j in range(8))

        def kv_part(head, p):
            b, h, slot = head // H, head % H, head % n_slots
            rows = [(p * part + r0, min(CH, part - r0)) for r0 in range(0, part, CH)]
            return [[(k_hbm.at[b, h, pl.ds(r, n)], kbuf.at[slot, pl.ds(r, n)], kvsem.at[0, slot], 0),
                     (v_hbm.at[b, h, pl.ds(r, n)], vbuf.at[slot, pl.ds(r, n)], kvsem.at[1, slot], 1)]
                    for r, n in rows]

        def kv_batch(step, streams):
            return _interleave(*[kv_part(step + LOOK + j, Q - 1 - j) for j in streams])

        j_mod = _pieces(wmod_hbm, wmod_v, sem_mod, 8, W_COLS * 3 // 4)
        j_q = _pieces(wq_hbm, wq_v, sem_q, 8, W_COLS)
        j_o = _pieces(wo_hbm, wo_v, sem_o, W_ROWS, D)
        j_g = _pieces(wg_hbm, wg_v, sem_g, W_ROWS, D)
        j_u = _pieces(wu_hbm, wu_v, sem_u, W_ROWS, D)
        j_d = []
        for t, (lo, hi) in enumerate(d_split):
            j_d += _pieces(wd_hbm.at[pl.ds(lo, hi - lo)], wd_v.at[pl.ds(lo, hi - lo)], dsem.at[t],
                           W_ROWS, D)

        def modulation():
            _wait_all(c_v, sem_c)
            _wait_all(wmod_v, sem_mod)
            cs = c_v[...].astype(F32)
            cs = (cs * _sigmoid(cs)).astype(BF16)
            mod_scr[...] = _dot(cs, wmod_v[...]).astype(BF16).astype(F32)

        def q_projection():
            _wait_all(x_v, sem_x)
            x = x_v[...].astype(F32)
            sa, ca = mod_scr[:, 0:D], mod_scr[:, D:2 * D]
            h1 = (_layernorm(x) * (1.0 + ca) + sa).astype(BF16)
            _wait_all(wq_v, sem_q)
            q = _dot(h1, wq_v[...]).astype(BF16)
            for h in range(H):
                q_scr[h] = q[:, h * Dh:(h + 1) * Dh]
            acc_scr[...] = jnp.zeros_like(acc_scr)

        def attend(head):
            b, h, slot = head // H, head % H, head % n_slots
            _wait_all(kbuf.at[slot], kvsem.at[0, slot])
            _wait_all(vbuf.at[slot], kvsem.at[1, slot])
            s = _dot_nt(q_scr[h], kbuf[slot])
            m = jnp.max(s, axis=1, keepdims=True)
            p = jnp.exp((s - m) * scale)
            l = jnp.sum(p, axis=1, keepdims=True)
            o = _dot(p.astype(BF16), vbuf[slot])
            row = jax.lax.broadcasted_iota(jnp.int32, (B, Dh), 0)
            o = jnp.where(row == b, o / l, 0.0).astype(BF16)
            acc_scr[...] += _dot(o, wo_v[pl.ds(pl.multiple_of(h * Dh, Dh), Dh), :])

        after = {}
        after[first] = [modulation, lambda: _issue(_halves(j_o))]
        after[first + 1] = [q_projection]
        after[-1] = [lambda: _wait_all(wo_v, sem_o)]
        after[n_heads - 4] = [lambda: _issue(_two_queues([], j_g))]
        after[n_heads - 3] = [lambda: _issue(_two_queues([], j_u))]
        after[n_heads - 2] = [lambda: _issue(_two_queues([], j_d))]

        _issue([[(c_hbm, c_v, sem_c, 0), (x_hbm, x_v, sem_x, 1)], [(wr_hbm, wr_v, sem_r, 0)]])
        _issue(_halves(j_mod))

        def step(it, carry):
            i = it + first

            @pl.when(it == 0)
            def _():
                _issue(_halves(j_q))

            @pl.when(i >= 0)
            def _():
                attend(i)

            for t in range(first, first + Q - 1):
                @pl.when(it == t - first)
                def _():
                    _issue(kv_batch(t, [j for j in range(Q) if t + LOOK + j >= 0]))

            @pl.when(jnp.logical_and(it >= Q - 1, it < n_main - first))
            def _():
                _issue(kv_batch(i, range(Q)))

            @pl.when(it == n_main - first)
            def _():
                for t in range(n_main, n_heads):
                    streams = [j for j in range(Q) if t + LOOK + j < n_heads]
                    if streams:
                        _issue(kv_batch(t, streams))

            for t in sorted(after):
                for action in after[t]:
                    pl.when(it == t - first)(action)
            return it

        last = jax.lax.fori_loop(0, n_heads - first, step, 0)

        ga, sb, cb, gb = (mod_scr[:, j * D:(j + 1) * D] for j in range(2, 6))
        x1 = x_v[...].astype(F32) + ga * acc_scr[...]
        h2 = _layernorm(x1) * (1.0 + cb) + sb
        h2b = h2.astype(BF16)
        _wait_all(wr_v, sem_r)
        r = jnp.sum(h2b.astype(F32) * wr_v[...].astype(F32).reshape(1, D), axis=-1, keepdims=True)
        _wait_all(wg_v, sem_g)
        _wait_all(wu_v, sem_u)
        g = _dot_nt(h2b, wg_v[...])
        u = _dot_nt(h2b, wu_v[...])
        a_scr[...] = (g * _sigmoid(g) * u).astype(BF16)
        acc_scr[...] = jnp.zeros_like(acc_scr)
        for t, (lo, hi) in enumerate(d_split):
            @pl.when(last >= 0)
            def _():
                _wait_all(wd_v.at[pl.ds(lo, hi - lo)], dsem.at[t])
                acc_scr[...] += _dot(a_scr[:, lo:hi], wd_v[lo:hi, :])

        upd = h2 * 0.0 + acc_scr[...] * _sigmoid(r)
        o_ref[...] = (x1 + gb * (h2 + upd)).astype(o_ref.dtype)

    scratch = [
        pltpu.VMEM((B, D), BF16),
        pltpu.VMEM((B, D), BF16),
        pltpu.VMEM((D,), BF16),
        pltpu.VMEM((D, 6 * D), BF16),
        pltpu.VMEM((D, H * Dh), BF16),
        pltpu.VMEM((H * Dh, D), BF16),
        pltpu.VMEM((F, D), BF16),
        pltpu.VMEM((F, D), BF16),
        pltpu.VMEM((F, D), BF16),
        pltpu.VMEM((n_slots, S, Dh), BF16),
        pltpu.VMEM((n_slots, S, Dh), BF16),
        pltpu.VMEM((H, B, Dh), BF16),
        pltpu.VMEM((B, 6 * D), F32),
        pltpu.VMEM((B, D), F32),
        pltpu.VMEM((B, F), BF16),
        pltpu.SemaphoreType.DMA((8,)),
        pltpu.SemaphoreType.DMA((2, n_slots)),
        pltpu.SemaphoreType.DMA((len(d_split),)),
    ]
    return kernel, scratch


@jax.jit
def pallas_adaLN_cond__gqa_block_cached__moe_arch_mod__decode_kernel(
    A_x: jax.Array,
    A_k_cache: jax.Array,
    A_v_cache: jax.Array,
    A_wq: jax.Array,
    A_wo: jax.Array,
    B_x: jax.Array,
    B_w_r: jax.Array,
    B_w_gate: jax.Array,
    B_w_up: jax.Array,
    B_w_down: jax.Array,
    c: jax.Array,
    w_mod: jax.Array,
):
    del B_x
    B, H, S, Dh = A_k_cache.shape
    D = A_x.shape[-1]
    F = B_w_gate.shape[-1]
    assert A_x.shape == (B, 1, D) and c.shape == (B, D) and S % Q == 0

    kernel, scratch = _make_kernel(B, H, S, Dh, D, F)
    hbm = pl.BlockSpec(memory_space=pltpu.HBM)
    out = pl.pallas_call(
        kernel,
        out_shape=jax.ShapeDtypeStruct((B, D), A_x.dtype),
        in_specs=[hbm] * 11,
        out_specs=pl.BlockSpec(memory_space=pltpu.VMEM),
        scratch_shapes=scratch,
        compiler_params=pltpu.CompilerParams(vmem_limit_bytes=100 * 1024 * 1024),
        name="adaln_gqa_moe_decode",
    )(A_x.reshape(B, D), c, w_mod, A_wq, A_wo, B_w_r, B_w_gate.T, B_w_up.T, B_w_down,
      A_k_cache, A_v_cache)
    return out.reshape(A_x.shape)
```

```python
import jax
import jax.numpy as jnp
import jax.experimental.pallas as pl
import jax.experimental.pallas.tpu as pltpu

F32 = jnp.float32
BF16 = jnp.bfloat16

Q = 4
STREAM_ORDER = (0, 2, 1, 3)
LOOK = 2
CH = 128
V_SKEW = 64
W_ROWS = 32
W_COLS = 2048
W_STREAMS = 4
D_CUTS = (1152,)
EPS = 1e-5


def _layernorm(x):
    m = jnp.mean(x, axis=-1, keepdims=True)
    xc = x - m
    v = jnp.mean(xc * xc, axis=-1, keepdims=True)
    return xc / jnp.sqrt(v + EPS)


def _sigmoid(x):
    return 1.0 / (1.0 + jnp.exp(-x))


def _dot(a, b):
    return jnp.dot(a, b, preferred_element_type=F32)


def _dot_nt(a, b):
    return jax.lax.dot_general(a, b, (((1,), (1,)), ((), ())), preferred_element_type=F32)


def _pieces(src, dst, sem, rows, cols):
    n_rows, n_cols = src.shape
    out = []
    for r0 in range(0, n_rows, rows):
        nr = min(rows, n_rows - r0)
        for c0 in range(0, n_cols, cols):
            nc = min(cols, n_cols - c0)
            if nc == n_cols:
                out.append((src.at[pl.ds(r0, nr)], dst.at[pl.ds(r0, nr)], sem))
            else:
                out.append((src.at[pl.ds(r0, nr), pl.ds(c0, nc)],
                            dst.at[pl.ds(r0, nr), pl.ds(c0, nc)], sem))
    return out


def _streams(jobs, n):
    per = -(-len(jobs) // n)
    return [jobs[s * per + t] for t in range(per) for s in range(n) if s * per + t < len(jobs)]


def _interleave(*lists):
    out = []
    for t in range(max(len(l) for l in lists)):
        for l in lists:
            if t < len(l):
                out.append(l[t])
    return out


def _two_queues(jobs0, jobs1):
    return _interleave([[j + (0,)] for j in jobs0], [[j + (1,)] for j in jobs1])


def _two_queues_grouped(jobs0, jobs1):
    n = max(len(jobs0), len(jobs1))
    return [[j[t] + (queue,) for queue, j in enumerate((jobs0, jobs1)) if t < len(j)] for t in range(n)]


def _halves(jobs):
    n = (len(jobs) + 1) // 2
    return _two_queues(_streams(jobs[:n], W_STREAMS), _streams(jobs[n:], W_STREAMS))


def _issue(groups):
    for group in groups:
        for src, dst, sem, queue in group:
            pltpu.make_async_copy(src, dst, sem).start(priority=queue)


def _wait_all(buf, sem):
    pltpu.make_async_copy(buf, buf, sem).wait()


def _make_kernel(B, H, S, Dh, D, F):
    n_heads = B * H
    part = S // Q
    n_slots = LOOK + Q - 1
    n_main = n_heads - n_slots
    first = -n_slots
    scale = Dh ** -0.5
    cuts = [0, *[c for c in D_CUTS if 0 < c < F], F]
    d_split = list(zip(cuts[:-1], cuts[1:]))

    def kernel(x_hbm, c_hbm, wmod_hbm, wq_hbm, wo_hbm, wr_hbm, wg_hbm, wu_hbm, wd_hbm, k_hbm, v_hbm,
               o_ref,
               x_v, c_v, wr_v, wmod_v, wq_v, wo_v, wg_v, wu_v, wd_v, kbuf, vbuf,
               q_scr, mod_scr, acc_scr, a_scr, wsem, kvsem, dsem):
        sem_c, sem_x, sem_r, sem_mod, sem_q, sem_o, sem_g, sem_u = (wsem.at[j] for j in range(8))

        def kv_part(head, p):
            b, h, slot = head // H, head % H, head % n_slots
            jobs = []
            for src, buf, queue, skew in ((k_hbm, kbuf, 0, 0), (v_hbm, vbuf, 1, V_SKEW)):
                edges = [0, *range(skew or CH, part, CH), part]
                rows = [(p * part + r0, r1 - r0) for r0, r1 in zip(edges[:-1], edges[1:])]
                jobs.append([(src.at[b, h, pl.ds(r, n)], buf.at[slot, pl.ds(r, n)], kvsem.at[queue, slot])
                             for r, n in rows])
            return _two_queues_grouped(*jobs)

        def kv_batch(step, streams):
            return _interleave(*[kv_part(step + LOOK + j, Q - 1 - j)
                                 for j in STREAM_ORDER if j in streams])

        j_mod = _pieces(wmod_hbm, wmod_v, sem_mod, 8, W_COLS * 3 // 4)
        j_q = _pieces(wq_hbm, wq_v, sem_q, 8, W_COLS)
        j_o = _pieces(wo_hbm, wo_v, sem_o, W_ROWS, D)
        j_g = _pieces(wg_hbm, wg_v, sem_g, W_ROWS, D)
        j_u = _pieces(wu_hbm, wu_v, sem_u, W_ROWS, D)
        j_d = []
        for t, (lo, hi) in enumerate(d_split):
            j_d += _pieces(wd_hbm.at[pl.ds(lo, hi - lo)], wd_v.at[pl.ds(lo, hi - lo)], dsem.at[t],
                           W_ROWS, D)

        def modulation():
            _wait_all(c_v, sem_c)
            _wait_all(wmod_v, sem_mod)
            cs = c_v[...].astype(F32)
            cs = (cs * _sigmoid(cs)).astype(BF16)
            mod_scr[...] = _dot(cs, wmod_v[...]).astype(BF16).astype(F32)

        def q_projection():
            _wait_all(x_v, sem_x)
            x = x_v[...].astype(F32)
            sa, ca = mod_scr[:, 0:D], mod_scr[:, D:2 * D]
            h1 = (_layernorm(x) * (1.0 + ca) + sa).astype(BF16)
            _wait_all(wq_v, sem_q)
            q = _dot(h1, wq_v[...]).astype(BF16)
            for h in range(H):
                q_scr[h] = q[:, h * Dh:(h + 1) * Dh]
            acc_scr[...] = jnp.zeros_like(acc_scr)

        def attend(head):
            b, h, slot = head // H, head % H, head % n_slots
            _wait_all(kbuf.at[slot], kvsem.at[0, slot])
            _wait_all(vbuf.at[slot], kvsem.at[1, slot])
            s = _dot_nt(q_scr[h], kbuf[slot])
            m = jnp.max(s, axis=1, keepdims=True)
            p = jnp.exp((s - m) * scale)
            l = jnp.sum(p, axis=1, keepdims=True)
            o = _dot(p.astype(BF16), vbuf[slot])
            row = jax.lax.broadcasted_iota(jnp.int32, (B, Dh), 0)
            o = jnp.where(row == b, o / l, 0.0).astype(BF16)
            acc_scr[...] += _dot(o, wo_v[pl.ds(pl.multiple_of(h * Dh, Dh), Dh), :])

        after = {}
        after[first] = [modulation, lambda: _issue(_halves(j_o))]
        after[first + 1] = [q_projection]
        after[-1] = [lambda: _wait_all(wo_v, sem_o)]
        after[n_heads - 4] = [lambda: _issue(_two_queues([], j_g))]
        after[n_heads - 3] = [lambda: _issue(_two_queues([], j_u))]
        after[n_heads - 2] = [lambda: _issue(_two_queues([], j_d))]

        _issue([[(c_hbm, c_v, sem_c, 0), (x_hbm, x_v, sem_x, 1)], [(wr_hbm, wr_v, sem_r, 0)]])
        _issue(_halves(j_mod))

        def step(it, carry):
            i = it + first

            @pl.when(it == 0)
            def _():
                _issue(_halves(j_q))

            @pl.when(i >= 0)
            def _():
                attend(i)

            for t in range(first, first + Q - 1):
                @pl.when(it == t - first)
                def _():
                    _issue(kv_batch(t, [j for j in range(Q) if t + LOOK + j >= 0]))

            @pl.when(jnp.logical_and(it >= Q - 1, it < n_main - first))
            def _():
                _issue(kv_batch(i, range(Q)))

            @pl.when(it == n_main - first)
            def _():
                for t in range(n_main, n_heads):
                    streams = [j for j in range(Q) if t + LOOK + j < n_heads]
                    if streams:
                        _issue(kv_batch(t, streams))

            for t in sorted(after):
                for action in after[t]:
                    pl.when(it == t - first)(action)
            return it

        last = jax.lax.fori_loop(0, n_heads - first, step, 0)

        ga, sb, cb, gb = (mod_scr[:, j * D:(j + 1) * D] for j in range(2, 6))
        x1 = x_v[...].astype(F32) + ga * acc_scr[...]
        h2 = _layernorm(x1) * (1.0 + cb) + sb
        h2b = h2.astype(BF16)
        _wait_all(wr_v, sem_r)
        r = jnp.sum(h2b.astype(F32) * wr_v[...].astype(F32).reshape(1, D), axis=-1, keepdims=True)
        _wait_all(wg_v, sem_g)
        _wait_all(wu_v, sem_u)
        g = _dot_nt(h2b, wg_v[...])
        u = _dot_nt(h2b, wu_v[...])
        a_scr[...] = (g * _sigmoid(g) * u).astype(BF16)
        acc_scr[...] = jnp.zeros_like(acc_scr)
        for t, (lo, hi) in enumerate(d_split):
            @pl.when(last >= 0)
            def _():
                _wait_all(wd_v.at[pl.ds(lo, hi - lo)], dsem.at[t])
                acc_scr[...] += _dot(a_scr[:, lo:hi], wd_v[lo:hi, :])

        upd = h2 * 0.0 + acc_scr[...] * _sigmoid(r)
        o_ref[...] = (x1 + gb * (h2 + upd)).astype(o_ref.dtype)

    scratch = [
        pltpu.VMEM((B, D), BF16),
        pltpu.VMEM((B, D), BF16),
        pltpu.VMEM((D,), BF16),
        pltpu.VMEM((D, 6 * D), BF16),
        pltpu.VMEM((D, H * Dh), BF16),
        pltpu.VMEM((H * Dh, D), BF16),
        pltpu.VMEM((F, D), BF16),
        pltpu.VMEM((F, D), BF16),
        pltpu.VMEM((F, D), BF16),
        pltpu.VMEM((n_slots, S, Dh), BF16),
        pltpu.VMEM((n_slots, S, Dh), BF16),
        pltpu.VMEM((H, B, Dh), BF16),
        pltpu.VMEM((B, 6 * D), F32),
        pltpu.VMEM((B, D), F32),
        pltpu.VMEM((B, F), BF16),
        pltpu.SemaphoreType.DMA((8,)),
        pltpu.SemaphoreType.DMA((2, n_slots)),
        pltpu.SemaphoreType.DMA((len(d_split),)),
    ]
    return kernel, scratch


@jax.jit
def pallas_adaLN_cond__gqa_block_cached__moe_arch_mod__decode_kernel(
    A_x: jax.Array,
    A_k_cache: jax.Array,
    A_v_cache: jax.Array,
    A_wq: jax.Array,
    A_wo: jax.Array,
    B_x: jax.Array,
    B_w_r: jax.Array,
    B_w_gate: jax.Array,
    B_w_up: jax.Array,
    B_w_down: jax.Array,
    c: jax.Array,
    w_mod: jax.Array,
):
    del B_x
    B, H, S, Dh = A_k_cache.shape
    D = A_x.shape[-1]
    F = B_w_gate.shape[-1]
    assert A_x.shape == (B, 1, D) and c.shape == (B, D) and S % Q == 0

    kernel, scratch = _make_kernel(B, H, S, Dh, D, F)
    hbm = pl.BlockSpec(memory_space=pltpu.HBM)
    out = pl.pallas_call(
        kernel,
        out_shape=jax.ShapeDtypeStruct((B, D), A_x.dtype),
        in_specs=[hbm] * 11,
        out_specs=pl.BlockSpec(memory_space=pltpu.VMEM),
        scratch_shapes=scratch,
        compiler_params=pltpu.CompilerParams(vmem_limit_bytes=100 * 1024 * 1024),
        name="adaln_gqa_moe_decode",
    )(A_x.reshape(B, D), c, w_mod, A_wq, A_wo, B_w_r, B_w_gate.T, B_w_up.T, B_w_down,
      A_k_cache, A_v_cache)
    return out.reshape(A_x.shape)
```
